```python
import os as _os
_os.environ.setdefault("JAX_PLATFORMS", "cpu")
import jax
import jax.numpy as jnp

def _softmax(x, axis=-1):
    return jax.nn.softmax(x, axis=axis)
def _gelu(x):
    return jax.nn.gelu(x, approximate=True)
def _silu(x):
    return jax.nn.silu(x)
def _sigmoid(x):
    return jax.nn.sigmoid(x)
def _layernorm(x, axis=-1, eps=1e-5):
    m = jnp.mean(x, axis=axis, keepdims=True)
    v = jnp.var(x, axis=axis, keepdims=True)
    return (x - m) / jnp.sqrt(v + eps)
def _scatter_add(tgt, idx, src, axis=0):
    return tgt.at[idx].add(src)
def _segment_sum(src, seg, n):
    return jax.ops.segment_sum(src, seg, n)
class _Rng:
    def __init__(self, key):
        self._k = key
    def _next(self):
        self._k, sub = jax.random.split(self._k)
        return sub
    def normal(self, shape):
        return jax.random.normal(self._next(), shape, dtype=jnp.bfloat16)
    def randint(self, lo, hi, shape):
        return jax.random.randint(self._next(), shape, lo, hi, dtype=jnp.int32)
    def uniform(self, shape, lo=0.0, hi=1.0):
        return jax.random.uniform(self._next(), shape, jnp.bfloat16, lo, hi)
    def permutation(self, n):
        return jax.random.permutation(self._next(), n)


kernel_name = 'concat_heads__ssm_conv_s4__grouped_kv_mqa__prompt'

def setup_inputs():
    _rng = _Rng(jax.random.key(int.from_bytes(__import__("os").urandom(4), "little")))
    _w = (lambda a: (lambda t: t.astype(jnp.bfloat16) if jnp.issubdtype(t.dtype, jnp.floating) else t)(jnp.asarray(a)))
    def _A_setup():
        B, L, D, N = 1, 2048, 448, 256
        A_re = -jnp.exp((lambda *s: _rng.normal(s) * 0.1)(D, N))
        A_im = jnp.pi * (lambda *s: _rng.normal(s) * 0.1)(D, N)
        B_re = (lambda *s: _rng.normal(s) * 0.1)(D, N)
        B_im = (lambda *s: _rng.normal(s) * 0.1)(D, N)
        C_re = (lambda *s: _rng.normal(s) * 0.1)(D, N)
        C_im = (lambda *s: _rng.normal(s) * 0.1)(D, N)
        log_dt = (lambda *s: _rng.normal(s) * 0.1)(D) * 0.5 - 4.0
        Dskip = (lambda *s: _rng.normal(s) * 0.05)(D)
        return {
            "u": _w((lambda *s: _rng.normal(s) * 0.05)(B, L, D)),
            "A_re": _w(A_re),
            "A_im": _w(A_im),
            "B_re": _w(B_re),
            "B_im": _w(B_im),
            "C_re": _w(C_re),
            "C_im": _w(C_im),
            "log_dt": _w(log_dt),
            "Dskip": _w(Dskip),
        }
    _A_in = _A_setup()

    def _B_setup():
        B, S, D, H = 1, 2048, 448, 16
        Dh = D // H
        return {
            "x": _w((lambda *s: _rng.normal(s) * 0.05)(B, S, D)),
            "wq": _w((lambda *s: _rng.normal(s) * 0.8)(D, H * Dh)),
            "wk": _w((lambda *s: _rng.normal(s) * 0.8)(D, Dh)),
            "wv": _w((lambda *s: _rng.normal(s) * 0.05)(D, Dh)),
            "wo": _w((lambda *s: _rng.normal(s) * 0.05)(H * Dh, D)),
        }
    _B_in = _B_setup()

    return {
        "A_u": _A_in["u"],
        "A_A_re": _A_in["A_re"],
        "A_A_im": _A_in["A_im"],
        "A_B_re": _A_in["B_re"],
        "A_B_im": _A_in["B_im"],
        "A_C_re": _A_in["C_re"],
        "A_C_im": _A_in["C_im"],
        "A_log_dt": _A_in["log_dt"],
        "A_Dskip": _A_in["Dskip"],
        "B_x": _B_in["x"],
        "B_wq": _B_in["wq"],
        "B_wk": _B_in["wk"],
        "B_wv": _B_in["wv"],
        "B_wo": _B_in["wo"],
    }

def reference(A_u, A_A_re, A_A_im, A_B_re, A_B_im, A_C_re, A_C_im, A_log_dt, A_Dskip, B_x, B_wq, B_wk, B_wv, B_wo):
    def _A_ref(u, A_re, A_im, B_re, B_im, C_re, C_im, log_dt, Dskip):
        Bsz, L, D = u.shape
        dt = jnp.exp(log_dt)[:, None]
        A = A_re + 1j * A_im
        Bc = B_re + 1j * B_im
        Cc = C_re + 1j * C_im
        logdA = dt * A
        dB = dt * Bc
        l = (lambda x, dt: x.astype(dt))(jnp.arange(L), A_re.dtype)
        P = jnp.exp(logdA[:, :, None] * l[None, None, :])
        K = jnp.einsum("dn,dnl,dn->dl", Cc, P, dB).real
        L2 = 2 * L
        Kp = jnp.pad(K, ((0, 0), (0, L)))
        up = (lambda x, *d: x.transpose(*d))(u, 0, 2, 1)
        up = jnp.pad(up, ((0, 0), (0, 0), (0, L)))
        Kf = (lambda x, axes=(-2,-1): jnp.fft.rfft2(x.astype(jnp.float32), axes=axes))(Kp[:, None, :], axes=(-2, -1))
        Uf = (lambda x, axes=(-2,-1): jnp.fft.rfft2(x.astype(jnp.float32), axes=axes))(up[:, :, None, :], axes=(-2, -1))
        Yf = Uf * Kf[None, :, :, :]
        y = (lambda x, s, axes=(-2,-1): jnp.fft.irfft2(x, s=s, axes=axes).astype(jnp.bfloat16))(Yf, (1, L2), axes=(-2, -1))[:, :, 0, :L]
        y = (lambda x, *d: x.transpose(*d))(y, 0, 2, 1) + u * Dskip[None, None, :]
        return y

    def _B_ref(x, wq, wk, wv, wo):
        B, S, D = x.shape
        H = 16
        Dh = D // H
        q = (lambda x, *d: x.transpose(*d))((x @ wq).reshape(B, S, H, Dh), 0, 2, 1, 3)
        k = x @ wk
        v = x @ wv
        scores = jnp.einsum("bhqd,bkd->bhqk", q, k) * (Dh ** -0.5)
        p = _softmax(scores, axis=-1)
        o = jnp.einsum("bhqk,bkd->bhqd", p, v)
        return (lambda x, *d: x.transpose(*d))(o, 0, 2, 1, 3).reshape(B, S, H * Dh) @ wo

    a = _A_ref(A_u, A_A_re, A_A_im, A_B_re, A_B_im, A_C_re, A_C_im, A_log_dt, A_Dskip)
    b = _B_ref(B_x, B_wq, B_wk, B_wv, B_wo)
    return jnp.concatenate([a, b], axis=-1)
```

```python
import functools
import itertools

import jax
import jax.numpy as jnp
import numpy as np
from jax import lax
import jax.experimental.pallas as pl
import jax.experimental.pallas.tpu as pltpu

L = 2048
D = 448
N = 256
H = 16
DH = D // H
NQ = 512
KC = 128
T = 128
NCH = L // T
NQB = L // NQ
NPAIR = NQB * H // 2
UNITS = D // 16
NKC = L // KC
X_CUTS = (0,384,896,2048)
PITCH = 9
PIN_LAGS = (2, 1, 2, 2)
F32 = jnp.float32
BF16 = jnp.bfloat16

HI = (1, 2, 3, 4, 258, 260, 516, 772, 1032, 1288, 1544, 1800)
CHUNK_TABLE = (0, 1, 2, 3, 4, 5, 5, 5, 6, 7, 7, 7, 8, 9, 9, 9)
CHUNK_MATRIX = (0, 1, 2, 3, 4, 5, 6, 7, 8, 9, 10, 11, 12, 9, 10, 11)


def _round_to_bf16(v):
    u = np.asarray(v, np.float32).view(np.uint32)
    return ((u + 0x7FFF + ((u >> 16) & 1)) & 0xFFFF0000).view(np.float32)


def _table_positions():
    lo = 4 * np.arange(64)
    pair = lambda a, b: np.concatenate([a + lo, b + lo])
    a0, a1, a2, a3, a4, a5 = [pair(HI[2 * i], HI[2 * i + 1]) for i in range(6)]
    lane = np.arange(128)
    low = (lane % 64) < 32
    t0, t1 = np.where(low, a0, np.roll(a1, 32)), np.where(low, np.roll(a0, 96), a1)
    keep = lambda k, prev, a: np.where(lane == k, prev, a)
    return [t0, keep(127, t0, t1), keep(127, a1, a2), a2, keep(127, a2, a3), a3,
            keep(127, a3, a4), a4, keep(126, a4, a5), a5]


def _dft_constants():
    t = np.arange(T)[:, None]
    w = 2.0 * np.pi * (np.arange(T)[None, :] + 0.5) / (2 * T)
    fwd = np.concatenate([np.cos(w * t), -np.sin(w * t)], axis=1)
    inv = np.concatenate([np.cos(w * t).T, -np.sin(w * t).T], axis=0) / T
    pos = _round_to_bf16(np.arange(L)).astype(np.int64)
    tables = _table_positions()
    mats = {}
    for m in range(NCH):
        lanes = tables[CHUNK_TABLE[m]]
        expand = np.zeros((T, T))
        for b in range(1 if m == 0 else 0, T):
            expand[np.nonzero(lanes == pos[m * T + b])[0][0], b] = 1.0
        mat = expand @ fwd
        assert np.array_equal(mats.setdefault(CHUNK_MATRIX[m], mat), mat)
    stack = np.stack([mats[i] for i in range(13)] + [fwd])
    return stack.astype(np.float32).astype(BF16), inv.astype(np.float32).astype(BF16)


_FWD_NP, _INV_NP = _dft_constants()


def _cmul(a, b):
    return a[0] * b[0] - a[1] * b[1], a[0] * b[1] + a[1] * b[0]


def _cmulc(a, b):
    return a[0] * b[0] + a[1] * b[1], a[1] * b[0] - a[0] * b[1]


def _csq(a):
    return (a[0] + a[1]) * (a[0] - a[1]), (a[0] + a[0]) * a[1]


def _column(vec_ref):
    row = vec_ref[...].astype(F32).reshape(1, D)
    row = jnp.concatenate([row, jnp.zeros((1, 512 - D), F32)], axis=1)
    return jnp.broadcast_to(row, (128, 512)).T[:D]


def _body(ut_hbm, are_hbm, aim_hbm, bre_hbm, bim_hbm, cre_hbm, cim_hbm, ldt_hbm, dsk_hbm,
          xt_hbm, wq_hbm, wkt_hbm, wvt_hbm, wo_hbm, fwd_hbm, inv_hbm,
          out_hbm,
          ldt_ref, dsk_ref, wkt_ref, wvt_ref, xt, ut, par, wq, wo, fwd, inv, wqt, wot, qw, kk, vv, s_bufs, raw,
          dt_col, dsk_col, k0_col, tabs, gbufs, ktab, kf, uf, yf, yt, stage,
          in_sem, out_sem):
    def x_copy(b):
        cols = pl.ds(X_CUTS[b], X_CUTS[b + 1] - X_CUTS[b])
        return pltpu.make_async_copy(xt_hbm.at[:, cols], xt.at[:, cols], in_sem.at[b])

    wq_copy = pltpu.make_async_copy(wq_hbm, wq, in_sem.at[4])
    par_sources = (are_hbm, aim_hbm, bre_hbm, bim_hbm, cre_hbm, cim_hbm)

    def par_copies(first, rows, sem):
        return [pltpu.make_async_copy(src.at[pl.ds(first, rows), :], par.at[i, pl.ds(first, rows), :],
                                      in_sem.at[sem + i]) for i, src in enumerate(par_sources)]

    par_head, par_rest = par_copies(0, 32, 19), par_copies(32, D - 32, 5)
    late_copies = [pltpu.make_async_copy(src, dst, in_sem.at[11 + i])
                   for i, (src, dst) in enumerate(((ut_hbm, ut), (fwd_hbm, fwd), (inv_hbm, inv), (wo_hbm, wo)))]
    small_copies = [pltpu.make_async_copy(src, dst, in_sem.at[15 + i]) for i, (src, dst) in enumerate(
        ((wkt_hbm, wkt_ref), (wvt_hbm, wvt_ref), (ldt_hbm, ldt_ref), (dsk_hbm, dsk_ref)))]
    for c in small_copies:
        c.start()
    wq_copy.start()
    x_copy(0).start()
    for c in par_head + [x_copy(b) for b in range(1, len(X_CUTS) - 1)] + par_rest + late_copies:
        c.start()

    def transposed(w_ref):
        w = w_ref[...]
        w = jnp.concatenate([w, jnp.zeros((D, 512 - D), BF16)], axis=1)
        w = jnp.concatenate([w, jnp.zeros((512 - D, 512), BF16)], axis=0)
        return w.T[:D, :D]

    for slot in range(4):
        xtab = tabs[slot][1]
        xtab[...] = jnp.zeros(xtab.shape, F32)
        for t in range(8):
            tabs[slot][0][t, 0:8, :] = jnp.full((8, 128), 1 - t % 2, F32)
    for slot in (2, 3):
        gbufs[slot][...] = jnp.zeros(gbufs[slot].shape, F32)
    for c in small_copies:
        c.wait()
    dt_col[...] = jnp.exp(_column(ldt_ref)).astype(BF16).astype(F32)
    dsk_col[...] = _column(dsk_ref)

    wq_copy.wait()
    wqt[2 * DH:, :] = transposed(wq).astype(F32)
    wqt[0:2 * DH, :] = jnp.concatenate([wkt_ref[...].astype(F32), wvt_ref[...].astype(F32)], axis=0)

    row32 = lax.broadcasted_iota(jnp.int32, (32, NQ), 0)
    q_scale = np.float32(DH ** -0.5 * np.log2(np.e))
    edges = sorted(set(X_CUTS) | set(range(0, L + 1, NQ)))
    for lo, hi in zip(edges, edges[1:]):
        if lo in X_CUTS:
            x_copy(X_CUTS.index(lo)).wait()
        if lo == X_CUTS[-2]:
            for c in par_head:
                c.wait()
        cols, n, row = slice(lo, hi), hi - lo, row32[:, :hi - lo]
        r = jnp.dot(wqt[...], xt[:, cols], preferred_element_type=F32)
        kt = jnp.where(row < DH, r[0:32], 0.0)
        vt = jnp.where(row >= 32 - DH, r[24:56], 0.0)
        pad = jnp.zeros((96, n), F32)
        kk[0, cols, :] = jnp.concatenate([kt, pad], axis=0).T[:, :32].astype(BF16)
        kk[1, cols, :] = jnp.concatenate([pltpu.roll(kt, 4, 0), pad], axis=0).T[:, :32].astype(BF16)
        vv[0, :, cols] = jnp.where(row == DH, 1.0, pltpu.roll(vt, DH, 0)).astype(BF16)
        vv[1, :, cols] = jnp.where(row == 0, 1.0, vt).astype(BF16)
        for hp in range(H // 2):
            even = jnp.where(row < DH, r[56 + 56 * hp:88 + 56 * hp] * q_scale, 0.0)
            odd = jnp.where(row >= 32 - DH, r[80 + 56 * hp:112 + 56 * hp] * q_scale, 0.0)
            for g, w in enumerate((even, odd)):
                qw[lo // NQ * H + 2 * hp + g, :, lo % NQ:lo % NQ + n] = w.astype(BF16)

    lane = lax.broadcasted_iota(jnp.int32, (8, 128), 1)

    def scores_chunk(c, parity, q, s_ref, m):
        rows = slice(c * KC, (c + 1) * KC)
        s = jnp.dot(kk[parity, rows, :], q, preferred_element_type=F32)
        s_ref[rows, :] = s
        mc = jnp.max(s.reshape(KC // 8, 8, NQ), axis=0)
        return mc if m is None else jnp.maximum(m, mc)

    def values_chunk(c, parity, s_ref, m, acc, cols=slice(None)):
        rows = slice(c * KC, (c + 1) * KC)
        p = jnp.exp2(s_ref[rows, cols].reshape(KC // 8, 8, -1) - m[None]).reshape(KC, -1).astype(BF16)
        a = jnp.dot(vv[parity, :, rows], p, preferred_element_type=F32)
        return a if acc is None else acc + a

    def interleave(main, side, side_items, pins=None):
        done = 0
        for i, piece in enumerate(main):
            piece()
            while done < side_items * (i + 1) // len(main):
                pinned = next(side)
                if pinned is not None and pins is not None:
                    pins.extend([pinned[0], v] for v in pinned[1])
                done += 1
        for _ in side:
            raise AssertionError("side work left over")

    def pair_pieces(pair, phase, m8, values=True):
        s_read, s_write = s_bufs[phase], s_bufs[1 - phase]
        state = {"m8": [None, None], "acc": [None, None], "m": [None, None], "q": [None, None], "pins": []}
        never = lane < -pair - 1

        def score(g, c):
            if c == 0:
                state["q"][g] = qw[2 * (pair + 1) + g]
            state["m8"][g] = scores_chunk(c, g, state["q"][g], s_write[g], state["m8"][g])

        def value(g, c):
            if c == 0:
                state["m"][g] = jnp.broadcast_to(jnp.max(m8[g], axis=0, keepdims=True), (8, NQ))
            for pin in state["pins"]:
                pin[0] -= 1
            for _, value in [pin for pin in state["pins"] if pin[0] == -1]:
                m = state["m"][g]
                state["m"][g] = jnp.concatenate(
                    [jnp.where(never, value, m[:, :128]), m[:, 128:]], axis=1)
            state["acc"][g] = values_chunk(c, g, s_read[g], state["m"][g], state["acc"][g])
            if c == NKC - 1:
                raw[2 * pair + g] = state["acc"][g]

        order = [(g, c) for g in range(2) for c in range(NKC)]
        sc = [functools.partial(score, g, c) for g, c in order]
        va = [functools.partial(value, g, c) for g, c in order]
        if not values:
            return sc, state
        return [sc[0], va[0]] + [p for both in zip(va[1:], sc[1:]) for p in both], state

    def run_steps(first, last, m8, make_side):
        def step(pair, phase, m8):
            pieces, state = pair_pieces(pair, phase, m8)
            interleave(pieces, *make_side(pair, phase), state["pins"])
            return tuple(state["m8"])

        def one(i, m8):
            return lax.cond(i % 2 == 0, lambda: step(i, 0, m8), lambda: step(i, 1, m8))
        return lax.fori_loop(first, last, one, m8)

    def power_tables(unit, slot):
        vtab, xtab, ztab = tabs[slot]
        rows = pl.ds(pl.multiple_of(unit * 16, 16), 16)
        for c in range(2):
            for nt in range(2):
                a_re, a_im, b_re, b_im, c_re, c_im = [
                    par[i, rows, 128 * nt:128 * nt + 128].astype(F32)[8 * c:8 * c + 8] for i in range(6)]
                dt = dt_col[pl.ds(pl.multiple_of(unit * 16 + 8 * c, 8), 8), :]
                t = (c * 2 + nt) * 2

                def put(ref, i, v):
                    if ref is xtab and c == 1:
                        i += 4
                    ref[t, PITCH * i:PITCH * i + 8, :] = v[0]
                    ref[t + 1, PITCH * i:PITCH * i + 8, :] = v[1]

                mag = jnp.exp(dt * a_re)
                ang = dt * a_im
                z1 = (mag * jnp.cos(ang), mag * jnp.sin(ang))
                yield z1
                w = _cmul((c_re, c_im), (dt * b_re, dt * b_im))
                x0 = (w[0], -w[1])
                k0 = w[0] if nt == 0 else k0 + w[0]
                if nt == 1:
                    k0_col[pl.ds(pl.multiple_of(unit * 16 + 8 * c, 8), 8), :] = k0
                x1 = _cmulc(x0, z1)
                put(xtab, 0, x1)
                z2 = _csq(z1)
                x2 = _cmulc(x0, z2)
                put(xtab, 1, x2)
                put(xtab, 2, _cmulc(x1, z2))
                x4 = _cmulc(x2, z2)
                put(xtab, 3, x4)
                z4 = _csq(z2)
                z8 = _csq(z4)
                z12 = _cmul(z8, z4)
                z16 = _csq(z8)
                yield x4 + z16
                for i, v in enumerate((z4, z8, z12, z16, _cmul(z16, z4), _cmul(z16, z8), _cmul(z16, z12))):
                    put(vtab, i + 1, v)
                z32 = _csq(z16)
                ztab[t] = z32[0]
                ztab[t + 1] = z32[1]
                z256 = _csq(_csq(_csq(z32)))
                put(xtab, 4, _cmulc(x2, z256))
                x = _cmulc(x4, z256)
                put(xtab, 5, x)
                yield x
                for i in range(6, 12):
                    x = _cmulc(x, z256 if i != 8 else _cmul(z256, z4))
                    put(xtab, i, x)
                yield x

    def kernel_values(slot):
        vtab, xtab, ztab = tabs[slot]
        for g in range(8):
            lhs, rhs = [], []
            for c in range(2):
                xs, vs = [[], []], [[], []]
                for nt in range(2):
                    t = (c * 2 + nt) * 2
                    step32 = tuple(jnp.broadcast_to(ztab[t + p, g:g + 1, :], (8, 128)) for p in range(2))
                    chain = [tuple(vtab[t + p, pl.ds(g, 8, stride=PITCH), :] for p in range(2))]
                    for _ in range(7):
                        chain.append(_cmul(chain[-1], step32))
                    for p in range(2):
                        vs[p].append(jnp.concatenate([w[p] for w in chain], axis=0))
                        xs[p].append(xtab[t + p, pl.ds(g, 16, stride=PITCH), :])
                    if c == 0 or nt == 0:
                        yield
                lhs.append(jnp.concatenate(xs[0] + xs[1], axis=1))
                rhs.append(jnp.concatenate(vs[0] + vs[1], axis=1))
            sub = lax.broadcasted_iota(jnp.int32, (8, 2 * N), 0)
            lhs = jnp.concatenate([lhs[0][:8], jnp.where(sub < 4, lhs[0][8:], lhs[1][:8]), lhs[1][8:]], axis=0)
            rhs = jnp.concatenate(rhs, axis=0).astype(BF16)

            def product(g=g, lhs=lhs, rhs=rhs):
                gbufs[slot][pl.ds(g, 24, stride=PITCH), :] = lax.dot_general(
                    lhs, rhs, (((1,), (1,)), ((), ())), preferred_element_type=F32)
            yield product

    def kernel_emit(unit, slot):
        halves = []
        for c in range(2):
            g = lambda i: gbufs[slot][(12 * c + i) * PITCH:(12 * c + i) * PITCH + 8, :]
            if c == 0:
                both = lambda i: jnp.where(lane < 64, g(i), pltpu.roll(g(i + 1), 64, 1))
            else:
                both = lambda i: jnp.where(lane < 64, pltpu.roll(g(i), 64, 1), g(i + 1))
            a0, a1, a2, a3, a4, a5 = [both(2 * i) for i in range(6)]
            low = (lane & 63) < 32
            t0, t1 = jnp.where(low, a0, pltpu.roll(a1, 32, 1)), jnp.where(low, pltpu.roll(a0, 96, 1), a1)
            keep = lambda k, prev, a: jnp.where(lane == k, prev, a)
            halves.append([t0, keep(127, t0, t1), keep(127, a1, a2), a2, keep(127, a2, a3), a3,
                           keep(127, a3, a4), a4, keep(126, a4, a5), a5])
            if c == 0:
                yield
        rows = pl.ds(pl.multiple_of(unit * 16, 16), 16)
        for i in range(10):
            ktab[i, rows, :] = jnp.concatenate([halves[0][i], halves[1][i]], axis=0).astype(BF16)
        yield

    def kernel_side(i, phase):
        other = 2 * (1 - phase)
        values = itertools.chain(*[kernel_values(2 * phase + j) for j in range(2)])
        tables = itertools.chain(*[
            power_tables(jnp.minimum(2 * i + 2 + j, UNITS - 2 + j), other + j) for j in range(2)])
        gather = itertools.chain(*[kernel_emit(jnp.maximum(2 * i - 2 + j, j), other + j) for j in range(2)])

        def run():
            product = None
            for n in range(64):
                pinned = (PIN_LAGS[n // 2 % 4], next(tables)) if n % 2 == 1 else None
                if n % 4 == 0 and product is not None:
                    product()
                product = next(values)
                if n % 16 == 7:
                    next(gather)
                if n == 63:
                    product()
                yield pinned
        return run(), 64

    def spectrum_side(item):
        def run():
            for grp in range(4):
                rows = pl.ds(pl.multiple_of(item * 32 + grp * 8, 8), 8)
                load = lambda ref, m: tuple(ref[m, rows, T * p:T * p + T] for p in range(3))
                for i0 in range(0, NCH, 2):
                    win, acc = {}, {}
                    for j in range(i0 + 2):
                        u = load(uf, j)
                        for i in (i0, i0 + 1):
                            if i >= j:
                                if i - j not in win:
                                    win[i - j] = load(kf, i - j)
                                t = tuple(a * b for a, b in zip(u, win[i - j]))
                                acc[i] = t if i not in acc else tuple(a + b for a, b in zip(acc[i], t))
                        if j % 2 == 1:
                            yield
                    for i in (i0, i0 + 1):
                        yf[i, rows, 0:T] = acc[i][0] - acc[i][2]
                        yf[i, rows, T:2 * T] = acc[i][0] + acc[i][1]
            yield
        return run(), 4 * 36 + 1

    def out_copy(first_row, rows, lo, hi, sem):
        window = (pl.ds(first_row, rows), pl.ds(lo, hi - lo))
        return pltpu.make_async_copy(stage.at[window], out_hbm.at[window], out_sem.at[sem])

    early_copies = [out_copy(0, L - NQ, 0, 2 * D, 0), out_copy(L - NQ, NQ, 0, 3 * T, 1)]
    last_copies = [out_copy(L - NQ + j * T, T, 3 * T, 2 * D, 2 + j) for j in range(NQ // T)]

    def normalised(even, odd):
        even = even * (1.0 / even[DH:DH + 1])
        odd = odd * (1.0 / odd[0:1])
        return [even[0:24], jnp.where(row32[:8, :even.shape[1]] < 4, even[24:32], odd[0:8]), odd[8:32]]

    def emit_columns(t, lo, hi, bt):
        parts = [yt[lo:min(hi, D), t * T:(t + 1) * T]] + ([bt] if hi > D else [])
        stage[t * T:(t + 1) * T, lo:hi] = jnp.concatenate(parts, axis=0).astype(BF16).T

    def emit_output(b):
        o = jnp.concatenate([p for hp in range(H // 2)
                             for p in normalised(raw[b * H + 2 * hp], raw[b * H + 2 * hp + 1])], axis=0).astype(BF16)
        bt = jnp.dot(wot[...], o, preferred_element_type=F32)
        for j in range(NQ // T):
            emit_columns(b * (NQ // T) + j, 0, 2 * D, bt[:, j * T:(j + 1) * T])

    pieces, state = pair_pieces(-1, 1, None, values=False)
    interleave(pieces, itertools.chain(power_tables(0, 0), power_tables(1, 1)), 32)
    m8 = tuple(state["m8"])

    for c in par_rest + late_copies:
        c.wait()
    kernel_steps = UNITS // 2
    m8 = run_steps(0, kernel_steps, m8, kernel_side)
    for j in range(2):
        for _ in kernel_emit(UNITS - 2 + j, 2 * ((kernel_steps - 1) % 2) + j):
            pass

    sign = jnp.where((lax.broadcasted_iota(jnp.int32, (64, T), 1) & 1) == 0, 1.0, -1.0).astype(F32)
    for r0 in range(0, D, 64):
        rows = slice(r0, r0 + 64)
        prev = None
        for m in range(NCH):
            cur = jnp.dot(ktab[CHUNK_TABLE[m], rows, :], fwd[CHUNK_MATRIX[m]], preferred_element_type=F32)
            re, im = cur[:, :T], cur[:, T:]
            if prev is not None:
                re, im = re - sign * prev[:, T:], im + sign * prev[:, :T]
            prev = cur
            kf[m, rows, :] = jnp.concatenate([re, im - re, re + im], axis=1)
            cur_u = jnp.dot(ut[rows, m * T:(m + 1) * T], fwd[13], preferred_element_type=F32)
            re, im = cur_u[:, :T], cur_u[:, T:]
            uf[m, rows, :] = jnp.concatenate([re + im, re, im], axis=1)
    spectrum_steps = D // 32
    m8 = run_steps(kernel_steps, kernel_steps + spectrum_steps, m8,
                   lambda i, phase: spectrum_side(i - kernel_steps))

    wot[...] = transposed(wo)
    skip = dsk_col[...] + jnp.sum(k0_col[...], axis=1, keepdims=True)
    for b in range(NQB):
        chunks = range(b * NQ // T, (b + 1) * NQ // T)
        for m in chunks:
            cols = slice(m * T, (m + 1) * T)
            y = jnp.dot(yf[m].astype(BF16), inv[...], preferred_element_type=F32)
            yt[:, cols] = y + ut[:, cols].astype(F32) * skip
        if b < NQB - 1:
            emit_output(b)
        else:
            for m in chunks:
                emit_columns(m, 0, 3 * T, None)
    for c in early_copies:
        c.start()

    m8 = run_steps(kernel_steps + spectrum_steps, NPAIR - 1, m8, lambda i, phase: (iter(()), 0))

    base = (NQB - 1) * H
    o = jnp.concatenate([p for hp in range(H // 2 - 1)
                         for p in normalised(raw[base + 2 * hp], raw[base + 2 * hp + 1])], axis=0)
    tops = [jnp.broadcast_to(jnp.max(m, axis=0, keepdims=True), (8, NQ)) for m in m8]

    def finish_columns(j, accs, bt):
        o_last = jnp.concatenate([o[3 * T:, j * T:(j + 1) * T]] + normalised(*accs), axis=0)
        bt = bt + jnp.dot(wot[:, 3 * T:], o_last.astype(BF16), preferred_element_type=F32)
        emit_columns((L - NQ) // T + j, 3 * T, 2 * D, bt)
        for done in {2: (0, 1, 2), 3: (3,)}.get(j, ()):
            last_copies[done].start()

    pending = None
    for j in range(NQ // T):
        cols = slice(j * T, (j + 1) * T)
        o_head = o[:3 * T, cols].astype(BF16)
        accs, bt = [None, None], []
        for n in range(2 * NKC):
            g, c = n % 2, n // 2
            accs[g] = values_chunk(c, g, s_bufs[(NPAIR - 1) % 2][g], tops[g][:, cols], accs[g], cols)
            if n == 14 and pending is not None:
                finish_columns(*pending)
            if n % 4 == 0 and len(bt) < D // 64:
                rows = slice(64 * len(bt), 64 * len(bt) + 64)
                bt.append(jnp.dot(wot[rows, :3 * T], o_head, preferred_element_type=F32))
        pending = (j, accs, jnp.concatenate(bt, axis=0))
    finish_columns(*pending)
    for c in early_copies + last_copies:
        c.wait()


@jax.jit
def pallas_concat_heads__ssm_conv_s4__grouped_kv_mqa__prompt_kernel(
    A_u: jax.Array,
    A_A_re: jax.Array,
    A_A_im: jax.Array,
    A_B_re: jax.Array,
    A_B_im: jax.Array,
    A_C_re: jax.Array,
    A_C_im: jax.Array,
    A_log_dt: jax.Array,
    A_Dskip: jax.Array,
    B_x: jax.Array,
    B_wq: jax.Array,
    B_wk: jax.Array,
    B_wv: jax.Array,
    B_wo: jax.Array,
):
    hbm = pl.BlockSpec(memory_space=pl.ANY)
    scratch = [
        pltpu.VMEM((D,), BF16),
        pltpu.VMEM((D,), BF16),
        pltpu.VMEM((DH, D), BF16),
        pltpu.VMEM((DH, D), BF16),
        pltpu.VMEM((D, L), BF16),
        pltpu.VMEM((D, L), BF16),
        pltpu.VMEM((6, D, N), BF16),
        pltpu.VMEM((D, D), BF16),
        pltpu.VMEM((D, D), BF16),
        pltpu.VMEM((14, T, 2 * T), BF16),
        pltpu.VMEM((2 * T, T), BF16),
        pltpu.VMEM((D + 2 * DH, D), F32),
        pltpu.VMEM((D, D), BF16),
        pltpu.VMEM((NQB * H, 32, NQ), BF16),
        pltpu.VMEM((2, L, 32), BF16),
        pltpu.VMEM((2, 32, L), BF16),
        [[pltpu.VMEM((L, NQ), F32)] * 2] * 2,
        pltpu.VMEM((NQB * H, 32, NQ), F32),
        pltpu.VMEM((D, 128), F32),
        pltpu.VMEM((D, 128), F32),
        pltpu.VMEM((D, 128), F32),
        [[pltpu.VMEM((8, 8 * PITCH, 128), F32), pltpu.VMEM((8, 16 * PITCH, 128), F32),
          pltpu.VMEM((8, 8, 128), F32)]] * 4,
        [pltpu.VMEM((32 * PITCH, 128), F32)] * 4,
        pltpu.VMEM((10, D, T), BF16),
        pltpu.VMEM((NCH, D, 3 * T), F32),
        pltpu.VMEM((NCH, D, 3 * T), F32),
        pltpu.VMEM((NCH, D, 2 * T), F32),
        pltpu.VMEM((D, L), F32),
        pltpu.VMEM((L, 2 * D), BF16),
        pltpu.SemaphoreType.DMA((25,)),
        pltpu.SemaphoreType.DMA((2 + NQ // T,)),
    ]
    out = pl.pallas_call(
        _body,
        out_shape=jax.ShapeDtypeStruct((L, 2 * D), BF16),
        in_specs=[hbm] * 16,
        out_specs=hbm,
        scratch_shapes=scratch,
        compiler_params=pltpu.CompilerParams(vmem_limit_bytes=100 * 2 ** 20),
    )(A_u[0].T, A_A_re, A_A_im, A_B_re, A_B_im, A_C_re, A_C_im, A_log_dt, A_Dskip,
      B_x[0].T, B_wq, B_wk.T, B_wv.T, B_wo, _FWD_NP, _INV_NP)
    return out[None]
```
